```python
import os as _os
_os.environ.setdefault("JAX_PLATFORMS", "cpu")
import jax
import jax.numpy as jnp

def _softmax(x, axis=-1):
    return jax.nn.softmax(x, axis=axis)
def _gelu(x):
    return jax.nn.gelu(x, approximate=True)
def _silu(x):
    return jax.nn.silu(x)
def _sigmoid(x):
    return jax.nn.sigmoid(x)
def _layernorm(x, axis=-1, eps=1e-5):
    m = jnp.mean(x, axis=axis, keepdims=True)
    v = jnp.var(x, axis=axis, keepdims=True)
    return (x - m) / jnp.sqrt(v + eps)
def _scatter_add(tgt, idx, src, axis=0):
    return tgt.at[idx].add(src)
def _segment_sum(src, seg, n):
    return jax.ops.segment_sum(src, seg, n)
class _Rng:
    def __init__(self, key):
        self._k = key
    def _next(self):
        self._k, sub = jax.random.split(self._k)
        return sub
    def normal(self, shape):
        return jax.random.normal(self._next(), shape, dtype=jnp.bfloat16)
    def randint(self, lo, hi, shape):
        return jax.random.randint(self._next(), shape, lo, hi, dtype=jnp.int32)
    def uniform(self, shape, lo=0.0, hi=1.0):
        return jax.random.uniform(self._next(), shape, jnp.bfloat16, lo, hi)
    def permutation(self, n):
        return jax.random.permutation(self._next(), n)


kernel_name = 'standalone__gqa_block_cached__near_ridge'

def setup_inputs():
    _rng = _Rng(jax.random.key(int.from_bytes(__import__("os").urandom(4), "little")))
    _w = (lambda a: (lambda t: t.astype(jnp.bfloat16) if jnp.issubdtype(t.dtype, jnp.floating) else t)(jnp.asarray(a)))
    B, Sq, D = 8, 80, 512
    Hq, Hkv, Sk, Dh = 32, 8, 2048, 128
    assert Hq % Hkv == 0, (Hq, Hkv)
    return {
        "x": _w((lambda *s: _rng.normal(s) * 0.8)(B, Sq, D)),
        "k_cache": _w((lambda *s: _rng.normal(s) * 0.8)(B, Hkv, Sk, Dh)),
        "v_cache": _w((lambda *s: _rng.normal(s) * 0.05)(B, Hkv, Sk, Dh)),
        "wq": _w((lambda *s: _rng.normal(s) * 0.8)(D, Hq * Dh) * (D ** -0.5)),
        "wo": _w((lambda *s: _rng.normal(s) * 0.05)(Hq * Dh, D) * ((Hq * Dh) ** -0.5)),
    }

def reference(x, k_cache, v_cache, wq, wo):
    B, Sq, D = x.shape
    Hq, Dh = 32, 128
    Hkv = k_cache.shape[1]
    rep = Hq // Hkv
    q = (lambda x, *d: x.transpose(*d))((x @ wq).reshape(B, Sq, Hq, Dh), 0, 2, 1, 3)
    k = jnp.repeat(k_cache, rep, axis=1)
    v = jnp.repeat(v_cache, rep, axis=1)
    scores = jnp.einsum("bhqd,bhkd->bhqk", q, k) * (Dh ** -0.5)
    p = _softmax(scores, axis=-1)
    o = jnp.einsum("bhqk,bhkd->bhqd", p, v)
    return (lambda x, *d: x.transpose(*d))(o, 0, 2, 1, 3).reshape(B, Sq, Hq * Dh) @ wo
```

```python
import math

import jax
import jax.numpy as jnp
from jax import lax
import jax.experimental.pallas as pl
import jax.experimental.pallas.tpu as pltpu

F32, BF16 = jnp.float32, jnp.bfloat16
LANES = 128
KB = 512


def _make_kernel(B, SQ, HKV, REP, SK, DH):
    HD = REP * DH
    HB = B // 2
    scale = (DH ** -0.5) * math.log2(math.e)

    def kernel(x_hbm, k_hbm, v_hbm, wq_hbm, wo_hbm, out_hbm,
               x_s, wq_s, wo_s, q_s, acc_s, out_s, k_s, v_s,
               x_sem, wq_sem, wo_sem, k_sem, v_sem, out_sem, fence_sem):

        def x_copy(half):
            rows = pl.ds(half * HB * SQ, HB * SQ)
            return pltpu.make_async_copy(x_hbm.at[rows], x_s.at[rows], x_sem.at[half])

        def wq_copy(h):
            return pltpu.make_async_copy(wq_hbm.at[:, pl.ds(h * HD, HD)], wq_s.at[h], wq_sem.at[h])

        def wo_copy(h):
            return pltpu.make_async_copy(wo_hbm.at[h], wo_s.at[h], wo_sem.at[h])

        def kv_copies(h, half):
            slot, bs = h % 2, pl.ds(half * HB, HB)
            return (pltpu.make_async_copy(k_hbm.at[bs, h], k_s.at[slot, bs], k_sem.at[slot, half]),
                    pltpu.make_async_copy(v_hbm.at[bs, h], v_s.at[slot, bs], v_sem.at[slot, half]))

        def out_copy(b0, nb, i):
            rows = pl.ds(b0 * SQ, nb * SQ)
            return pltpu.make_async_copy(out_s.at[rows], out_hbm.at[rows], out_sem.at[i])

        def start_head(h):
            for c in kv_copies(h, 0) + kv_copies(h, 1):
                c.start()
            wo_copy(h).start()

        def fence():
            pl.semaphore_signal(fence_sem, 1)
            pl.semaphore_wait(fence_sem, 1)

        q_groups = ((1, 2), tuple(range(3, HKV)))
        x_copy(0).start()
        wq_copy(0).start()
        fence()
        x_copy(1).start()
        for hs in q_groups:
            fence()
            for h in hs:
                wq_copy(h).start()
        fence()
        for c in kv_copies(0, 0):
            c.start()
        wo_copy(0).start()
        fence()
        for c in kv_copies(0, 1):
            c.start()
        fence()
        start_head(1)
        acc_s[...] = jnp.zeros_like(acc_s)

        def q_proj(h, b0, nb):
            q = jnp.dot(x_s[pl.ds(b0 * SQ, nb * SQ), :], wq_s[h], preferred_element_type=F32)
            q = (q * scale).astype(BF16)
            for i in range(nb):
                for r in range(REP):
                    q_s[h, b0 + i, r * SQ:(r + 1) * SQ, :] = q[i * SQ:(i + 1) * SQ, r * DH:(r + 1) * DH]

        wq_copy(0).wait()

        def first_q(half, carry):
            x_copy(half).wait()
            q_proj(0, pl.multiple_of(half * HB, HB), HB)
            return carry

        lax.fori_loop(0, 2, first_q, 0)
        for hs in q_groups:
            for h in hs:
                wq_copy(h).wait()
            for h in hs:
                q_proj(h, 0, B)

        def attend(h, b0, nb, is_last=None):
            slot = h % 2
            scores, outs = {}, {}

            def qk(i):
                s = lax.dot_general(q_s[h, b0 + i], k_s[slot, b0 + i], (((1,), (1,)), ((), ())),
                                    preferred_element_type=F32)
                m = s[:, 0:LANES]
                for t in range(1, SK // LANES):
                    m = jnp.maximum(m, s[:, t * LANES:(t + 1) * LANES])
                scores[i] = (s, jnp.max(m, axis=-1, keepdims=True))

            def pv(i, midway=None):
                s, m = scores.pop(i)
                l = o = None
                for j in range(SK // KB):
                    if midway is not None and j == 2:
                        midway()
                    mj = m if o is None else jnp.maximum(m, jnp.minimum(m, o))
                    ps = []
                    for t in range(j * KB // LANES, (j + 1) * KB // LANES):
                        p = jnp.exp2(s[:, t * LANES:(t + 1) * LANES] - mj)
                        l = p if l is None else l + p
                        ps.append(p)
                    ps[-1] = jnp.minimum(ps[-1], l)
                    p = jnp.concatenate(ps, axis=1).astype(BF16)
                    oj = jnp.dot(p, v_s[slot, b0 + i, j * KB:(j + 1) * KB, :], preferred_element_type=F32)
                    o = oj if o is None else o + oj
                l = jnp.sum(l, axis=-1, keepdims=True)
                r = pl.reciprocal(l, approx=True)
                r = r * (2.0 - l * r)
                o = (o * r).astype(BF16)
                outs[i] = jnp.concatenate([o[u * SQ:(u + 1) * SQ, :] for u in range(REP)], axis=1)

            def out_proj(*ii):
                o = jnp.concatenate([outs.pop(i) for i in ii], axis=0)
                rows = pl.ds(pl.multiple_of((b0 + ii[0]) * SQ, SQ), len(ii) * SQ)
                y = acc_s[rows, :] + jnp.dot(o, wo_s[h], preferred_element_type=F32)
                acc_s[rows, :] = y
                if is_last is not None:
                    out_s[rows, :] = y.astype(BF16)

            for i in range(nb):
                qk(i)
                midway = None
                if is_last is not None and i == nb - 1:
                    pl.when(is_last)(lambda: out_copy(0, B - 3, 0).start())
                    midway = lambda: pl.when(is_last)(lambda: out_copy(B - 3, 1, 1).start())
                if i >= 2:
                    out_proj(i - 2)
                pv(i, midway)
            out_proj(nb - 2, nb - 1)

        wo_copy(0).wait()

        def first_head(half, carry):
            for c in kv_copies(0, half):
                c.wait()
            attend(0, half * HB, HB)
            return carry

        lax.fori_loop(0, 2, first_head, 0)

        def head(h, carry):
            for c in kv_copies(h, 0) + kv_copies(h, 1):
                c.wait()
            wo_copy(h).wait()
            pl.when(h + 1 < HKV)(lambda: start_head(h + 1))
            attend(h, 0, B, is_last=h == HKV - 1)
            return carry

        lax.fori_loop(1, HKV, head, 0)
        out_copy(B - 2, 2, 2).start()
        out_copy(0, B - 3, 0).wait()
        out_copy(B - 3, 1, 1).wait()
        out_copy(B - 2, 2, 2).wait()

    return kernel


@jax.jit
def pallas_standalone__gqa_block_cached__near_ridge_kernel(
    x: jax.Array,
    k_cache: jax.Array,
    v_cache: jax.Array,
    wq: jax.Array,
    wo: jax.Array,
):
    B, SQ, D = x.shape
    _, HKV, SK, DH = k_cache.shape
    REP = wq.shape[1] // (HKV * DH)
    HD = REP * DH

    out = pl.pallas_call(
        _make_kernel(B, SQ, HKV, REP, SK, DH),
        in_specs=[pl.BlockSpec(memory_space=pl.ANY)] * 5,
        out_specs=pl.BlockSpec(memory_space=pl.ANY),
        out_shape=jax.ShapeDtypeStruct((B * SQ, D), BF16),
        scratch_shapes=[
            pltpu.VMEM((B * SQ, D), BF16),
            pltpu.VMEM((HKV, D, HD), BF16),
            pltpu.VMEM((HKV, HD, D), BF16),
            pltpu.VMEM((HKV, B, REP * SQ, DH), BF16),
            pltpu.VMEM((B * SQ, D), F32),
            pltpu.VMEM((B * SQ, D), BF16),
            pltpu.VMEM((2, B, SK, DH), BF16),
            pltpu.VMEM((2, B, SK, DH), BF16),
            pltpu.SemaphoreType.DMA((2,)),
            pltpu.SemaphoreType.DMA((HKV,)),
            pltpu.SemaphoreType.DMA((HKV,)),
            pltpu.SemaphoreType.DMA((2, 2)),
            pltpu.SemaphoreType.DMA((2, 2)),
            pltpu.SemaphoreType.DMA((3,)),
            pltpu.SemaphoreType.REGULAR,
        ],
        compiler_params=pltpu.CompilerParams(vmem_limit_bytes=100 * 1024 * 1024),
    )(x.reshape(B * SQ, D), k_cache, v_cache, wq, wo.reshape(HKV, HD, D))
    return out.reshape(B, SQ, D)
```

```python
import math

import jax
import jax.numpy as jnp
from jax import lax
import jax.experimental.pallas as pl
import jax.experimental.pallas.tpu as pltpu

F32, BF16 = jnp.float32, jnp.bfloat16
LANES = 128
KB = 512
LAG = 2


def _make_kernel(B, SQ, D, HKV, REP, SK, DH):
    HD = REP * DH
    HB = B // 2
    scale = (DH ** -0.5) * math.log2(math.e)
    SEM_X, SEM_WQ, SEM_WO, SEM_K, SEM_V = 0, 2, 4, 6, 6 + B

    def kernel(x_hbm, k_hbm, v_hbm, wq_hbm, wo_hbm, out_hbm,
               x_s, w_s, acc_s, out_s, k_s, v_s, in_sem, out_sem, fence_sem):

        def x_copy(half):
            rows = pl.ds(half * HB * SQ, HB * SQ)
            return pltpu.make_async_copy(x_hbm.at[rows], x_s.at[rows], in_sem.at[SEM_X + half])

        def wq_copy(h, c):
            cols = pl.ds(h * HD + c * (HD // 2), HD // 2)
            return pltpu.make_async_copy(wq_hbm.at[:, cols], w_s.at[h & 1, c], in_sem.at[SEM_WQ + c])

        def wo_copy(h, c):
            rows, cols = pl.ds(h * HD, HD), pl.ds(c * (D // 2), D // 2)
            return pltpu.make_async_copy(wo_hbm.at[rows, cols], w_s.at[h & 1, 2 + c], in_sem.at[SEM_WO + c])

        def k_copy(h, b, n):
            bs = pl.ds(b, n)
            return pltpu.make_async_copy(k_hbm.at[bs, h], k_s.at[h & 1, bs], in_sem.at[SEM_K + b])

        def v_copy(h, b, n):
            bs = pl.ds(b, n)
            return pltpu.make_async_copy(v_hbm.at[bs, h], v_s.at[h & 1, bs], in_sem.at[SEM_V + b])

        def out_copy(b, n, col=0, ncols=D):
            rows, cols = pl.ds(b * SQ, n * SQ), pl.ds(col, ncols)
            return pltpu.make_async_copy(out_s.at[rows, cols], out_hbm.at[rows, cols], out_sem)

        first = [x_copy(0), wq_copy(0, 0), wq_copy(0, 1), x_copy(1)]
        for b in range(B):
            first.append(k_copy(0, b, 1))
            if b == LAG:
                first += [wo_copy(0, 0), wo_copy(0, 1)]
            first.append(v_copy(0, b, 1))
        for copy in first:
            copy.start()
            pl.semaphore_signal(fence_sem, 1)
            pl.semaphore_wait(fence_sem, 1)
        acc_s[...] = jnp.zeros_like(acc_s)
        x_copy(0).wait()

        def head(h, carry):
            slot = h & 1
            is_last = h == HKV - 1
            qs, scores, outs = {}, {}, {}

            def prefetch(copy, *where):
                pl.when(h + 1 < HKV)(lambda: copy(h + 1, *where).start())

            def wait_kv(copy, i):
                pl.when(h == 0)(lambda: copy(h, i, 1).wait())
                if i % HB == 0:
                    pl.when(h > 0)(lambda: copy(h, i, HB).wait())

            def q_proj(half, c):
                x = x_s[half * HB * SQ:(half + 1) * HB * SQ, :]
                q = (jnp.dot(x, w_s[slot, c], preferred_element_type=F32) * scale).astype(BF16)
                for i in range(HB):
                    for r in range(REP // 2):
                        qs[half * HB + i, c * (REP // 2) + r] = q[i * SQ:(i + 1) * SQ, r * DH:(r + 1) * DH]

            def qk(i):
                q = jnp.concatenate([qs.pop((i, r)) for r in range(REP)], axis=0)
                s = lax.dot_general(q, k_s[slot, i], (((1,), (1,)), ((), ())), preferred_element_type=F32)
                m = s[:, 0:LANES]
                for t in range(1, SK // LANES):
                    m = jnp.maximum(m, s[:, t * LANES:(t + 1) * LANES])
                scores[i] = (s, jnp.max(m, axis=-1, keepdims=True))

            def pv(i, midway):
                s, m = scores.pop(i)
                l = o = None
                for j in range(SK // KB):
                    if midway is not None and j == SK // KB // 2:
                        midway()
                    mj = m if o is None else jnp.maximum(m, jnp.minimum(m, o))
                    ps = []
                    for t in range(j * KB // LANES, (j + 1) * KB // LANES):
                        p = jnp.exp2(s[:, t * LANES:(t + 1) * LANES] - mj)
                        l = p if l is None else l + p
                        ps.append(p)
                    ps[-1] = jnp.minimum(ps[-1], l)
                    p = jnp.concatenate(ps, axis=1).astype(BF16)
                    oj = jnp.dot(p, v_s[slot, i, j * KB:(j + 1) * KB, :], preferred_element_type=F32)
                    o = oj if o is None else o + oj
                l = jnp.sum(l, axis=-1, keepdims=True)
                inv = pl.reciprocal(l, approx=True)
                inv = inv * (2.0 - l * inv)
                o = (o * inv).astype(BF16)
                outs[i] = jnp.concatenate([o[r * SQ:(r + 1) * SQ, :] for r in range(REP)], axis=1)

            def out_proj(b, n, send_left=False):
                o = jnp.concatenate([outs.pop(i) for i in range(b, b + n)], axis=0)
                rows = slice(b * SQ, (b + n) * SQ)
                halves = (slice(0, D // 2), slice(D // 2, D))
                ys = [acc_s[rows, cols] + jnp.dot(o, w_s[slot, 2 + c], preferred_element_type=F32)
                      for c, cols in enumerate(halves)]
                for c, cols in enumerate(halves):
                    if send_left and c == 1:
                        pl.when(is_last)(lambda: out_copy(b, n, 0, D // 2).start())
                    acc_s[rows, cols] = ys[c]
                    out_s[rows, cols] = ys[c].astype(BF16)

            wq_copy(h, 0).wait()
            q_proj(0, 0)
            prefetch(wq_copy, 0)
            wq_copy(h, 1).wait()
            q_proj(0, 1)
            prefetch(wq_copy, 1)
            pl.when(h == 0)(lambda: x_copy(1).wait())
            q_proj(1, 0)
            q_proj(1, 1)
            prefetch(wo_copy, 0)
            prefetch(wo_copy, 1)

            for i in range(B):
                wait_kv(k_copy, i)
                qk(i)
                if i % HB == HB - 1:
                    prefetch(k_copy, i - HB + 1, HB)
                midway = None
                if i == B - 1:
                    pl.when(is_last)(lambda: out_copy(0, B - LAG - 1).start())
                    midway = lambda: pl.when(is_last)(lambda: out_copy(B - LAG - 1, 1).start())
                if i == LAG:
                    wo_copy(h, 0).wait()
                    wo_copy(h, 1).wait()
                if i >= LAG:
                    out_proj(i - LAG, 1)
                wait_kv(v_copy, i)
                pv(i, midway)
                if i % HB == HB - 1:
                    prefetch(v_copy, i - HB + 1, HB)
            out_proj(B - LAG, LAG, send_left=True)
            return carry

        lax.fori_loop(0, HKV, head, 0)
        out_copy(B - LAG, LAG, D // 2, D // 2).start()
        out_copy(0, B).wait()

    return kernel


@jax.jit
def pallas_standalone__gqa_block_cached__near_ridge_kernel(
    x: jax.Array,
    k_cache: jax.Array,
    v_cache: jax.Array,
    wq: jax.Array,
    wo: jax.Array,
):
    B, SQ, D = x.shape
    _, HKV, SK, DH = k_cache.shape
    REP = wq.shape[1] // (HKV * DH)
    assert REP * DH == D

    out = pl.pallas_call(
        _make_kernel(B, SQ, D, HKV, REP, SK, DH),
        in_specs=[pl.BlockSpec(memory_space=pl.ANY)] * 5,
        out_specs=pl.BlockSpec(memory_space=pl.ANY),
        out_shape=jax.ShapeDtypeStruct((B * SQ, D), BF16),
        scratch_shapes=[
            pltpu.VMEM((B * SQ, D), BF16),
            pltpu.VMEM((2, 4, D, D // 2), BF16),
            pltpu.VMEM((B * SQ, D), F32),
            pltpu.VMEM((B * SQ, D), BF16),
            pltpu.VMEM((2, B, SK, DH), BF16),
            pltpu.VMEM((2, B, SK, DH), BF16),
            pltpu.SemaphoreType.DMA((6 + 2 * B,)),
            pltpu.SemaphoreType.DMA,
            pltpu.SemaphoreType.REGULAR,
        ],
        compiler_params=pltpu.CompilerParams(
            vmem_limit_bytes=64 * 1024 * 1024,
            disable_bounds_checks=True,
            disable_semaphore_checks=True,
            flags={"XLA_TPU_RESCHEDULE_DMA_DONES": True},
        ),
    )(x.reshape(B * SQ, D), k_cache, v_cache, wq, wo)
    return out.reshape(B, SQ, D)
```

```python
import math

import jax
import jax.numpy as jnp
from jax import lax
import jax.experimental.pallas as pl
import jax.experimental.pallas.tpu as pltpu

F32, BF16 = jnp.float32, jnp.bfloat16
LANES = 128
KB = 512
LAG = 2


def _make_kernel(B, SQ, D, HKV, REP, SK, DH):
    HD = REP * DH
    HB = B // 2
    scale = (DH ** -0.5) * math.log2(math.e)
    SEM_X, SEM_WQ, SEM_WO, SEM_K, SEM_V = 0, 2, 4, 8, 8 + B

    def kernel(x_hbm, k_hbm, v_hbm, wq_hbm, wo_hbm, out_hbm,
               x_s, w_s, acc_s, out_s, k_s, v_s, in_sem, out_sem, fence_sem):

        def x_copy(half):
            rows = pl.ds(half * HB * SQ, HB * SQ)
            return pltpu.make_async_copy(x_hbm.at[rows], x_s.at[rows], in_sem.at[SEM_X + half])

        def wq_copy(h, c):
            cols = pl.ds(h * HD + c * (HD // 2), HD // 2)
            return pltpu.make_async_copy(wq_hbm.at[:, cols], w_s.at[h & 1, c], in_sem.at[SEM_WQ + c])

        def wo_copy(h, c):
            rows, cols = pl.ds(h * HD, HD), pl.ds(c * (D // 2), D // 2)
            sem = in_sem.at[SEM_WO + 2 * (h & 1) + c]
            return pltpu.make_async_copy(wo_hbm.at[rows, cols], w_s.at[h & 1, 2 + c], sem)

        def k_copy(h, b, n):
            bs = pl.ds(b, n)
            return pltpu.make_async_copy(k_hbm.at[bs, h], k_s.at[h & 1, bs], in_sem.at[SEM_K + b])

        def v_copy(h, b, n):
            bs = pl.ds(b, n)
            return pltpu.make_async_copy(v_hbm.at[bs, h], v_s.at[h & 1, bs], in_sem.at[SEM_V + b])

        def out_copy(b, n, col=0, ncols=D):
            rows, cols = pl.ds(b * SQ, n * SQ), pl.ds(col, ncols)
            return pltpu.make_async_copy(out_s.at[rows, cols], out_hbm.at[rows, cols], out_sem)

        first = [x_copy(0), wq_copy(0, 0), wq_copy(0, 1), x_copy(1)]
        for b in range(B):
            first.append(k_copy(0, b, 1))
            if b == LAG:
                first += [wo_copy(0, 0), wo_copy(0, 1)]
            first.append(v_copy(0, b, 1))
        for copy in first:
            copy.start()
            pl.semaphore_signal(fence_sem, 1)
            pl.semaphore_wait(fence_sem, 1)
        acc_s[...] = jnp.zeros_like(acc_s)
        x_copy(0).wait()

        def head(h, carry):
            slot = h & 1
            is_last = h == HKV - 1
            qs, scores, outs = {}, {}, {}

            def prefetch(copy, *where):
                pl.when(h + 1 < HKV)(lambda: copy(h + 1, *where).start())

            def wait_kv(copy, i):
                pl.when(h == 0)(lambda: copy(h, i, 1).wait())
                if i % HB == 0:
                    pl.when(h > 0)(lambda: copy(h, i, HB).wait())

            def q_proj(half, c):
                x = x_s[half * HB * SQ:(half + 1) * HB * SQ, :]
                q = (jnp.dot(x, w_s[slot, c], preferred_element_type=F32) * scale).astype(BF16)
                for i in range(HB):
                    for r in range(REP // 2):
                        qs[half * HB + i, c * (REP // 2) + r] = q[i * SQ:(i + 1) * SQ, r * DH:(r + 1) * DH]

            def qk(i):
                q = jnp.concatenate([qs.pop((i, r)) for r in range(REP)], axis=0)
                s = lax.dot_general(q, k_s[slot, i], (((1,), (1,)), ((), ())), preferred_element_type=F32)
                m = s[:, 0:LANES]
                for t in range(1, SK // LANES):
                    m = jnp.maximum(m, s[:, t * LANES:(t + 1) * LANES])
                scores[i] = (s, jnp.max(m, axis=-1, keepdims=True))

            def pv(i, midway):
                s, m = scores.pop(i)
                l = o = None
                for j in range(SK // KB):
                    if midway is not None and j == SK // KB // 2:
                        midway()
                    mj = m if o is None else jnp.maximum(m, jnp.minimum(m, o))
                    ps = []
                    for t in range(j * KB // LANES, (j + 1) * KB // LANES):
                        p = jnp.exp2(s[:, t * LANES:(t + 1) * LANES] - mj)
                        l = p if l is None else l + p
                        ps.append(p)
                    ps[-1] = jnp.minimum(ps[-1], l)
                    p = jnp.concatenate(ps, axis=1).astype(BF16)
                    oj = jnp.dot(p, v_s[slot, i, j * KB:(j + 1) * KB, :], preferred_element_type=F32)
                    o = oj if o is None else o + oj
                l = jnp.sum(l, axis=-1, keepdims=True)
                inv = pl.reciprocal(l, approx=True)
                inv = inv * (2.0 - l * inv)
                o = (o * inv).astype(BF16)
                outs[i] = jnp.concatenate([o[r * SQ:(r + 1) * SQ, :] for r in range(REP)], axis=1)

            def out_proj(b, n, send_left=False):
                o = jnp.concatenate([outs.pop(i) for i in range(b, b + n)], axis=0)
                rows = slice(b * SQ, (b + n) * SQ)
                halves = (slice(0, D // 2), slice(D // 2, D))
                ys = [acc_s[rows, cols] + jnp.dot(o, w_s[slot, 2 + c], preferred_element_type=F32)
                      for c, cols in enumerate(halves)]
                for c, cols in enumerate(halves):
                    if send_left and c == 1:
                        pl.when(is_last)(lambda: out_copy(b, n, 0, D // 2).start())
                    acc_s[rows, cols] = ys[c]
                    out_s[rows, cols] = ys[c].astype(BF16)

            wq_copy(h, 0).wait()
            q_proj(0, 0)
            prefetch(wq_copy, 0)
            wq_copy(h, 1).wait()
            q_proj(0, 1)
            prefetch(wq_copy, 1)
            pl.when(h == 0)(lambda: x_copy(1).wait())
            q_proj(1, 0)
            q_proj(1, 1)
            prefetch(wo_copy, 0)
            prefetch(wo_copy, 1)

            for i in range(B):
                wait_kv(k_copy, i)
                qk(i)
                if i % HB == HB - 1:
                    prefetch(k_copy, i - HB + 1, HB)
                midway = None
                if i == B - 1:
                    pl.when(is_last)(lambda: out_copy(0, B - LAG - 1).start())
                    midway = lambda: pl.when(is_last)(lambda: out_copy(B - LAG - 1, 1).start())
                if i == LAG:
                    wo_copy(h, 0).wait()
                    wo_copy(h, 1).wait()
                if i >= LAG:
                    out_proj(i - LAG, 1)
                wait_kv(v_copy, i)
                pv(i, midway)
                if i % HB == HB - 1:
                    prefetch(v_copy, i - HB + 1, HB)
            out_proj(B - LAG, LAG, send_left=True)
            return carry

        lax.fori_loop(0, HKV, head, 0)
        out_copy(B - LAG, LAG, D // 2, D // 2).start()
        out_copy(0, B).wait()

    return kernel


@jax.jit
def pallas_standalone__gqa_block_cached__near_ridge_kernel(
    x: jax.Array,
    k_cache: jax.Array,
    v_cache: jax.Array,
    wq: jax.Array,
    wo: jax.Array,
):
    B, SQ, D = x.shape
    _, HKV, SK, DH = k_cache.shape
    REP = wq.shape[1] // (HKV * DH)
    assert REP * DH == D

    out = pl.pallas_call(
        _make_kernel(B, SQ, D, HKV, REP, SK, DH),
        in_specs=[pl.BlockSpec(memory_space=pl.ANY)] * 5,
        out_specs=pl.BlockSpec(memory_space=pl.ANY),
        out_shape=jax.ShapeDtypeStruct((B * SQ, D), BF16),
        scratch_shapes=[
            pltpu.VMEM((B * SQ, D), BF16),
            pltpu.VMEM((2, 4, D, D // 2), BF16),
            pltpu.VMEM((B * SQ, D), F32),
            pltpu.VMEM((B * SQ, D), BF16),
            pltpu.VMEM((2, B, SK, DH), BF16),
            pltpu.VMEM((2, B, SK, DH), BF16),
            pltpu.SemaphoreType.DMA((8 + 2 * B,)),
            pltpu.SemaphoreType.DMA,
            pltpu.SemaphoreType.REGULAR,
        ],
        compiler_params=pltpu.CompilerParams(
            vmem_limit_bytes=64 * 1024 * 1024,
            disable_bounds_checks=True,
            disable_semaphore_checks=True,
            flags={"XLA_TPU_RESCHEDULE_DMA_DONES": True},
        ),
    )(x.reshape(B * SQ, D), k_cache, v_cache, wq, wo)
    return out.reshape(B, SQ, D)
```
